```python
import jax
import jax.numpy as jnp

def _softmax(x, axis=-1):
    return jax.nn.softmax(x, axis=axis)
def _gelu(x):
    return jax.nn.gelu(x, approximate=True)
def _silu(x):
    return jax.nn.silu(x)
def _sigmoid(x):
    return jax.nn.sigmoid(x)
def _layernorm(x, axis=-1, eps=1e-5):
    m = jnp.mean(x, axis=axis, keepdims=True)
    v = jnp.var(x, axis=axis, keepdims=True)
    return (x - m) / jnp.sqrt(v + eps)
def _scatter_add(tgt, idx, src, axis=0):
    return tgt.at[idx].add(src)
def _segment_sum(src, seg, n):
    return jax.ops.segment_sum(src, seg, n)
class _Rng:
    def __init__(self, key):
        self._k = key
    def _next(self):
        self._k, sub = jax.random.split(self._k)
        return sub
    def normal(self, shape):
        return jax.random.normal(self._next(), shape, dtype=jnp.bfloat16)
    def randint(self, lo, hi, shape):
        return jax.random.randint(self._next(), shape, lo, hi, dtype=jnp.int32)
    def uniform(self, shape, lo=0.0, hi=1.0):
        return jax.random.uniform(self._next(), shape, jnp.bfloat16, lo, hi)
    def permutation(self, n):
        return jax.random.permutation(self._next(), n)


kernel_name = 'recurrent_scan__sliding_local_dilated__swiglu_ffn__prompt'

def setup_inputs():
    _rng = _Rng(jax.random.key(int.from_bytes(__import__("os").urandom(4), "little")))
    _w = (lambda a: (lambda t: t.astype(jnp.bfloat16) if jnp.issubdtype(t.dtype, jnp.floating) else t)(jnp.asarray(a)))
    def _A_setup():
        B, S, D = 1, 2048, 1024
        return {
            "x": _w((lambda *s: _rng.normal(s) * 0.05)(B, S, D)),
            "wqkv": _w((lambda *s: _rng.normal(s) * 0.05)(D, 3 * D)),
            "wo": _w((lambda *s: _rng.normal(s) * 0.05)(D, D)),
        }
    _A_in = _A_setup()

    def _B_setup():
        B, S, D, F = 1, 2048, 1024, 3584
        return {
            "x": _w((lambda *s: _rng.normal(s) * 0.05)(B, S, D)),
            "w_gate": _w((lambda *s: _rng.normal(s) * 0.05)(D, F)),
            "w_up": _w((lambda *s: _rng.normal(s) * 0.05)(D, F)),
            "w_down": _w((lambda *s: _rng.normal(s) * 0.05)(F, D)),
        }
    _B_in = _B_setup()

    return {
        "A_x": _A_in["x"],
        "A_wqkv": _A_in["wqkv"],
        "A_wo": _A_in["wo"],
        "B_x": _B_in["x"],
        "B_w_gate": _B_in["w_gate"],
        "B_w_up": _B_in["w_up"],
        "B_w_down": _B_in["w_down"],
    }

def reference(A_x, A_wqkv, A_wo, B_x, B_w_gate, B_w_up, B_w_down):
    def _A_ref(x, wqkv, wo):
        B, S, D = x.shape
        H = 32; Dh = D // H
        W, dil = 8, 2
        qkv = (lambda x, *d: x.transpose(*d))((x @ wqkv).reshape(B, S, 3, H, Dh), 2, 0, 3, 1, 4)
        q, k, v = qkv[0], qkv[1], qkv[2]
        scale = Dh ** -0.5
        pos = jnp.arange(S)
        off = jnp.arange(W) * dil
        idx = pos[:, None] - off[None, :]
        mask = idx >= 0
        idx_c = jnp.where(mask, idx, 0).reshape(-1)
        kg = k[:, :, idx_c, :].reshape(B, H, S, W, Dh)
        vg = v[:, :, idx_c, :].reshape(B, H, S, W, Dh)
        logits = jnp.einsum("bhsd,bhswd->bhsw", q, kg) * scale
        logits = jnp.where(mask[None, None, :, :], logits, -1e9)
        attn = _softmax(logits, axis=-1)
        o = jnp.einsum("bhsw,bhswd->bhsd", attn, vg)
        return (lambda x, *d: x.transpose(*d))(o, 0, 2, 1, 3).reshape(B, S, D) @ wo

    def _B_ref(x, w_gate, w_up, w_down):
        g = _silu(x @ w_gate)
        u = x @ w_up
        return (g * u) @ w_down

    x = A_x
    xn = _layernorm(x, axis=-1)
    s = _A_ref(xn, A_wqkv, A_wo)
    g = _silu(_B_ref(xn, B_w_gate, B_w_up, B_w_down))
    return x + s * g
```

```python
import functools
import numpy as np
import jax
import jax.numpy as jnp
from jax import lax
import jax.experimental.pallas as pl
import jax.experimental.pallas.tpu as pltpu

BM = 512
FC = 512
FA = 4
WST = 2
USE_PERM = False
PERM_G = 4
NSEP = 2

def _lane_swap(a, b, bit, lane):
    hi = (lane & bit) != 0
    na = jnp.where(hi, pltpu.roll(b, bit, 1), a)
    nb = jnp.where(hi, b, pltpu.roll(a, 128 - bit, 1))
    return na, nb

def _sub_swap(a, b, bit, sub):
    hi = (sub & bit) != 0
    na = jnp.where(hi, pltpu.roll(b, bit, 0), a)
    nb = jnp.where(hi, b, pltpu.roll(a, 8 - bit, 0))
    return na, nb

def _sigmoid(x):
    return 0.5 * jnp.tanh(0.5 * x) + 0.5

def kernel(x_hbm, wqkv_hbm, wo_hbm, wg_hbm, wu_hbm, wd_hbm, out_hbm,
           x_v, xnA, xnB, wqkv_v, wqkvp_v, wo_v, wop_v, wg_v, wu_v, wd_v,
           q_v, k_v, v_v, o_v, acc_v, accF_v, out_v,
           sep_v, sem_in, sem_o, sem_s):
    S, D = x_v.shape
    F = wg_v.shape[1]
    NB = S // BM
    NF = F // FC
    f32 = jnp.float32
    bf16 = jnp.bfloat16

    copies = {}
    order = [("x", 0)]
    for f in range(NF):
        if 1 <= f <= 3:
            order += [("qkv", f - 1)]
        if f == 4:
            order += [("wo", 0)]
        order += [("g", f), ("u", f), ("d", f)]
        if f == 4:
            order += [("x", 1), ("x", 2), ("x", 3)]
    for n, (kind, j) in enumerate(order):
        if kind == "x":
            src, dst = x_hbm.at[pl.ds(j * BM, BM), :], x_v.at[pl.ds(j * BM, BM), :]
        elif kind == "g":
            src, dst = wg_hbm.at[:, pl.ds(j * FC, FC)], wg_v.at[:, pl.ds(j * FC, FC)]
        elif kind == "u":
            src, dst = wu_hbm.at[:, pl.ds(j * FC, FC)], wu_v.at[:, pl.ds(j * FC, FC)]
        elif kind == "d":
            src, dst = wd_hbm.at[pl.ds(j * FC, FC), :], wd_v.at[pl.ds(j * FC, FC), :]
        elif kind == "qkv":
            src, dst = wqkv_hbm.at[:, pl.ds(j * D, D)], wqkv_v.at[:, pl.ds(j * D, D)]
        else:
            src, dst = wo_hbm, wo_v
        copies[(kind, j)] = pltpu.make_async_copy(src, dst, sem_in.at[n])
    for key in order:
        copies[key].start()

    def out_copy(row0, n=BM, off=0):
        return pltpu.make_async_copy(out_v.at[pl.ds(off, n), :], out_hbm.at[pl.ds(row0, n), :], sem_o.at[0])

    lane = lax.broadcasted_iota(jnp.int32, (8, 128), 1)
    sub = lax.broadcasted_iota(jnp.int32, (8, 128), 0)

    def perm_qkv(j):
        for rg in range(0, D // 16, PERM_G):
            strips = []
            for r in range(rg, rg + PERM_G):
                strips.append([pltpu.bitcast(wqkv_v[pl.ds(r * 16, 16), pl.ds(j * D + c * 128, 128)], jnp.uint32) for c in range(8)])
            for (cb, lb) in ((4, 16), (2, 8), (1, 4)):
                for cols in strips:
                    for c in range(8):
                        if c & cb == 0:
                            cols[c], cols[c | cb] = _lane_swap(cols[c], cols[c | cb], lb, lane)
            for k_, cols in enumerate(strips):
                for c in range(8):
                    wqkvp_v[pl.ds((rg + k_) * 16, 16), pl.ds(j * D + c * 128, 128)] = pltpu.bitcast(cols[c], bf16)

    def perm_wo():
        for g in range(16):
            h4 = (g >> 3) & 1; h10 = (g >> 1) & 3; d4 = g & 1
            for c in range(8):
                tl = []
                for h32 in range(4):
                    t = h4 * 32 + h32 * 8 + h10 * 2 + d4
                    tl.append(pltpu.bitcast(wo_v[pl.ds(t * 16, 16), pl.ds(c * 128, 128)], jnp.uint32))
                tl[0], tl[2] = _sub_swap(tl[0], tl[2], 4, sub)
                tl[1], tl[3] = _sub_swap(tl[1], tl[3], 4, sub)
                tl[0], tl[1] = _sub_swap(tl[0], tl[1], 2, sub)
                tl[2], tl[3] = _sub_swap(tl[2], tl[3], 2, sub)
                for d32 in range(4):
                    tn = d4 * 32 + d32 * 8 + h10 * 2 + h4
                    wop_v[pl.ds(tn * 16, 16), pl.ds(c * 128, 128)] = pltpu.bitcast(tl[d32], bf16)

    scale = 32.0 ** -0.5

    def layernorm(row0):
        xb = x_v[pl.ds(row0, BM), :].astype(f32)
        mu = jnp.mean(xb, axis=-1, keepdims=True)
        xc = xb - mu
        var = jnp.mean(xc * xc, axis=-1, keepdims=True)
        xnA[...] = (xc * lax.rsqrt(var + 1e-5)).astype(bf16)

    def ffn_chunk(f, xn, pre=lambda kind: None):
        pre("g")
        g = jnp.dot(xn[...], wg_v[:, pl.ds(f * FC, FC)], preferred_element_type=f32)
        pre("u")
        u = jnp.dot(xn[...], wu_v[:, pl.ds(f * FC, FC)], preferred_element_type=f32)
        h = (g * _sigmoid(g) * u).astype(bf16)
        pre("d")
        dn = jnp.dot(h, wd_v[pl.ds(f * FC, FC), :], preferred_element_type=f32)
        if f == 0:
            acc_v[...] = dn
        elif f == NF - 1:
            accF_v[...] = acc_v[...] + dn
        else:
            acc_v[...] += dn

    def qkv():
        for j, ref in enumerate((q_v, k_v, v_v)):
            off = 0 if j == 0 else 16
            for c2 in range(4):
                t = jnp.dot(xnA[...], wqkvp_v[:, pl.ds(j * D + c2 * 256, 256)], preferred_element_type=f32)
                if j == 0:
                    t = t * scale
                ref[2 * c2, pl.ds(off, BM), :] = t[:, :128]
                ref[2 * c2 + 1, pl.ds(off, BM), :] = t[:, 128:]
        xnB[...] = xnA[...]

    def att_piece(r0, row0):
        R = 8
        b0 = (lane & 1) != 0
        b1 = (lane & 2) != 0
        def swp(a, bit):
            if USE_PERM:
                return jnp.take_along_axis(a, lane ^ bit, axis=1)
            return jnp.where(b0 if bit == 1 else b1, pltpu.roll(a, bit, 1), pltpu.roll(a, 128 - bit, 1))
        qs = [q_v[c, pl.ds(r0, R), :] for c in range(8)]
        lg = []
        for w0 in range(0, 8, WST):
            grp = []
            for w in range(w0, w0 + WST):
                a = None
                for c in range(8):
                    t = qs[c] * k_v[c, pl.ds(r0 + 16 - 2 * w, R), :]
                    a = t if a is None else a + t
                grp.append(a)
            r1 = [swp(a, 1) for a in grp]
            grp = [a + b for a, b in zip(grp, r1)]
            r2 = [swp(a, 2) for a in grp]
            grp = [a + b for a, b in zip(grp, r2)]
            lg += grp
        if row0 + r0 < 16:
            rows = (row0 + r0) + sub
            lg = [a if w == 0 else jnp.where(rows >= 2 * w, a, -1e9) for w, a in enumerate(lg)]
        m = lg[0]
        for w in range(1, 8):
            m = jnp.maximum(m, lg[w])
        p = [jnp.exp(l - m) for l in lg]
        ssum = p[0]
        for w in range(1, 8):
            ssum = ssum + p[w]
        inv = 1.0 / ssum
        p = [pw * inv for pw in p]
        for c in range(8):
            o = None
            for w in range(8):
                t = p[w] * v_v[c, pl.ds(r0 + 16 - 2 * w, R), :]
                o = t if o is None else o + t
            o_v[pl.ds(r0, R), pl.ds(c * 128, 128)] = o.astype(bf16)

    def wo_epi(row0):
        s = jnp.dot(o_v[...], wop_v[...], preferred_element_type=f32)
        a = accF_v[...]
        res = x_v[pl.ds(row0, BM), :].astype(f32) + s * (a * _sigmoid(a))
        out_v[...] = res.astype(bf16)

    k_v[:, 0:16, :] = jnp.zeros((8, 16, 128), f32)
    v_v[:, 0:16, :] = jnp.zeros((8, 16, 128), f32)

    nsep = [0]
    seps = [pltpu.make_async_copy(x_hbm.at[pl.ds(0, 16), pl.ds(0, 128)], sep_v.at[n], sem_s.at[n]) for n in range(NSEP)]
    for c in seps:
        c.start()
    def sep():
        seps[nsep[0]].wait()
        nsep[0] += 1

    if True:
        copies[("x", 0)].wait()
        layernorm(0)

    if True:
        for f in range(FA):
            if 1 <= f <= 3:
                copies[("qkv", f - 1)].wait()
            if f == 0:
                ffn_chunk(f, xnA, lambda kind: copies[(kind, 0)].wait())
            else:
                for kind in ("g", "u", "d"):
                    copies[(kind, f)].wait()
                ffn_chunk(f, xnA)
            if 1 <= f <= 3:
                perm_qkv(f - 1)
        copies[("wo", 0)].wait()
        qkv()
        perm_wo()

    for i in range(NB):
        row0 = i * BM
        if True:
            if i == 0:
                for f in range(FA, NF):
                    for kind in ("g", "u", "d"):
                        copies[(kind, f)].wait()
            if i + 1 < NB:
                copies[("x", i + 1)].wait()
            else:
                sep()
            for f in range(FA, NF):
                ffn_chunk(f, xnB)
            for t in range(BM // 8):
                att_piece(t * 8, row0)
            if i + 1 < NB:
                layernorm(row0 + BM)
        if True:
            if i >= 1:
                out_copy(row0 - BM).wait()
            else:
                sep()
            if i + 1 < NB:
                k_v[:, pl.ds(0, 16), :] = k_v[:, pl.ds(BM, 16), :]
                v_v[:, pl.ds(0, 16), :] = v_v[:, pl.ds(BM, 16), :]
            wo_epi(row0)
            out_copy(row0).start()
            if i + 1 < NB:
                for f in range(FA):
                    ffn_chunk(f, xnA)
                qkv()
    out_copy(S - BM).wait()


@jax.jit
def pallas_recurrent_scan__sliding_local_dilated__swiglu_ffn__prompt_kernel(
    A_x, A_wqkv, A_wo, B_x, B_w_gate, B_w_up, B_w_down):
    B, S, D = A_x.shape
    F = B_w_gate.shape[1]
    x2 = A_x.reshape(S, D)
    bf = jnp.bfloat16
    f32 = jnp.float32
    NB = S // BM
    NF = F // FC
    out = pl.pallas_call(
        kernel,
        out_shape=jax.ShapeDtypeStruct((S, D), bf),
        in_specs=[pl.BlockSpec(memory_space=pl.ANY)] * 6,
        out_specs=pl.BlockSpec(memory_space=pl.ANY),
        scratch_shapes=[
            pltpu.VMEM((S, D), bf), pltpu.VMEM((BM, D), bf), pltpu.VMEM((BM, D), bf),
            pltpu.VMEM((D, 3 * D), bf), pltpu.VMEM((D, 3 * D), bf),
            pltpu.VMEM((D, D), bf), pltpu.VMEM((D, D), bf),
            pltpu.VMEM((D, F), bf), pltpu.VMEM((D, F), bf), pltpu.VMEM((F, D), bf),
            pltpu.VMEM((8, BM, 128), f32),
            pltpu.VMEM((8, BM + 16, 128), f32),
            pltpu.VMEM((8, BM + 16, 128), f32),
            pltpu.VMEM((BM, D), bf), pltpu.VMEM((BM, D), f32), pltpu.VMEM((BM, D), f32),
            pltpu.VMEM((BM, D), bf),
            pltpu.VMEM((NSEP, 16, 128), bf),
            pltpu.SemaphoreType.DMA((NB + 4 + 3 * NF,)), pltpu.SemaphoreType.DMA((1,)), pltpu.SemaphoreType.DMA((NSEP,)),
        ],
        compiler_params=pltpu.CompilerParams(vmem_limit_bytes=110 * 1024 * 1024),
    )(x2, A_wqkv, A_wo, B_w_gate, B_w_up, B_w_down)
    return out.reshape(B, S, D)
```

```python
import functools
import numpy as np
import jax
import jax.numpy as jnp
from jax import lax
import jax.experimental.pallas as pl
import jax.experimental.pallas.tpu as pltpu

BM = 512
FC = 512
FA = 4
WST = 2
USE_PERM = False
PERM_G = 2
LN_G = 16
X0P = 4
NSEP = 2
NB_GEN = 4
PWO = 'qk0'
TC = 256
G0_PIECES = ((0, 128), (128, 128), (256, 256))

def _lane_swap(a, b, bit, lane):
    hi = (lane & bit) != 0
    na = jnp.where(hi, pltpu.roll(b, bit, 1), a)
    nb = jnp.where(hi, b, pltpu.roll(a, 128 - bit, 1))
    return na, nb

def _sub_swap(a, b, bit, sub):
    hi = (sub & bit) != 0
    na = jnp.where(hi, pltpu.roll(b, bit, 0), a)
    nb = jnp.where(hi, b, pltpu.roll(a, 8 - bit, 0))
    return na, nb

def _sigmoid(x):
    return 0.5 * jnp.tanh(0.5 * x) + 0.5

def kernel(x_hbm, wqkv_hbm, wo_hbm, wg_hbm, wu_hbm, wd_hbm, out_hbm,
           x_v, xnA, xnB, wqkv_v, wqkvp_v, wo_v, wop_v, wg_v, wu_v, wd_v,
           q_v, k_v, v_v, o_v, acc_v, accF_v, out_v,
           sep_v, sem_in, sem_o, sem_s):
    S, D = x_v.shape
    F = wg_v.shape[1]
    NB = S // BM
    NF = F // FC
    f32 = jnp.float32
    bf16 = jnp.bfloat16

    copies = {}
    order = [("x0", p) for p in range(X0P)] + [("g0", 0), ("g0", 1), ("g0", 2), ("u", 0), ("d", 0)]
    for f in range(1, FA):
        if f >= 2:
            order += [("qkv", f - 2)]
        order += [("g", f), ("u", f), ("d", f)]
    order += [("qkv", 2), ("wo", 0), ("x", 1)]
    for f in range(FA, NF):
        order += [("g", f), ("u", f), ("d", f)]
    order += [("x", j) for j in range(2, NB)]
    for n, (kind, j) in enumerate(order):
        if kind == "x0":
            rs = pl.ds(j * (BM // X0P), BM // X0P)
            src, dst = x_hbm.at[rs, :], x_v.at[rs, :]
        elif kind == "x":
            src, dst = x_hbm.at[pl.ds(j * BM, BM), :], x_v.at[pl.ds(j * BM, BM), :]
        elif kind == "g0":
            c0, cn = G0_PIECES[j]
            src, dst = wg_hbm.at[:, pl.ds(c0, cn)], wg_v.at[:, pl.ds(c0, cn)]
        elif kind == "g":
            src, dst = wg_hbm.at[:, pl.ds(j * FC, FC)], wg_v.at[:, pl.ds(j * FC, FC)]
        elif kind == "u":
            src, dst = wu_hbm.at[:, pl.ds(j * FC, FC)], wu_v.at[:, pl.ds(j * FC, FC)]
        elif kind == "d":
            src, dst = wd_hbm.at[pl.ds(j * FC, FC), :], wd_v.at[pl.ds(j * FC, FC), :]
        elif kind == "qkv":
            src, dst = wqkv_hbm.at[:, pl.ds(j * D, D)], wqkv_v.at[:, pl.ds(j * D, D)]
        else:
            src, dst = wo_hbm, wo_v
        copies[(kind, j)] = pltpu.make_async_copy(src, dst, sem_in.at[n])
    for key in order:
        copies[key].start()

    def out_copy(row0):
        return pltpu.make_async_copy(out_v, out_hbm.at[pl.ds(row0, BM), :], sem_o.at[0])

    def out_copy_cols(row0, j):
        cs = pl.ds(j * TC, TC)
        return pltpu.make_async_copy(out_v.at[:, cs], out_hbm.at[pl.ds(row0, BM), cs], sem_o.at[1 + j])

    lane = lax.broadcasted_iota(jnp.int32, (8, 128), 1)
    sub = lax.broadcasted_iota(jnp.int32, (8, 128), 0)

    def perm_qkv(j):
        for rg in range(0, D // 16, PERM_G):
            strips = []
            for r in range(rg, rg + PERM_G):
                strips.append([pltpu.bitcast(wqkv_v[pl.ds(r * 16, 16), pl.ds(j * D + c * 128, 128)], jnp.uint32) for c in range(8)])
            for (cb, lb) in ((4, 16), (2, 8), (1, 4)):
                for cols in strips:
                    for c in range(8):
                        if c & cb == 0:
                            cols[c], cols[c | cb] = _lane_swap(cols[c], cols[c | cb], lb, lane)
            for k_, cols in enumerate(strips):
                for c in range(8):
                    wqkvp_v[pl.ds((rg + k_) * 16, 16), pl.ds(j * D + c * 128, 128)] = pltpu.bitcast(cols[c], bf16)

    def perm_wo():
        for g in range(16):
            h4 = (g >> 3) & 1; h10 = (g >> 1) & 3; d4 = g & 1
            for c in range(8):
                tl = []
                for h32 in range(4):
                    t = h4 * 32 + h32 * 8 + h10 * 2 + d4
                    tl.append(pltpu.bitcast(wo_v[pl.ds(t * 16, 16), pl.ds(c * 128, 128)], jnp.uint32))
                tl[0], tl[2] = _sub_swap(tl[0], tl[2], 4, sub)
                tl[1], tl[3] = _sub_swap(tl[1], tl[3], 4, sub)
                tl[0], tl[1] = _sub_swap(tl[0], tl[1], 2, sub)
                tl[2], tl[3] = _sub_swap(tl[2], tl[3], 2, sub)
                for d32 in range(4):
                    tn = d4 * 32 + d32 * 8 + h10 * 2 + h4
                    wop_v[pl.ds(tn * 16, 16), pl.ds(c * 128, 128)] = pltpu.bitcast(tl[d32], bf16)

    scale = 32.0 ** -0.5

    def ln_rows(src0, dst, dst0, n):
        xb = x_v[pl.ds(src0, n), :].astype(f32)
        mu = jnp.mean(xb, axis=-1, keepdims=True)
        xc = xb - mu
        var = jnp.mean(xc * xc, axis=-1, keepdims=True)
        dst[pl.ds(dst0, n), :] = (xc * lax.rsqrt(var + 1e-5)).astype(bf16)

    def layernorm(row0, dst):
        for r in range(0, BM, LN_G):
            ln_rows(row0 + r, dst, r, LN_G)

    def ffn_chunk(f, xn, first=False):
        if first:
            gs = []
            for j, (c0, cn) in enumerate(G0_PIECES):
                copies[("g0", j)].wait()
                gs.append(jnp.dot(xn[...], wg_v[:, pl.ds(c0, cn)], preferred_element_type=f32))
            g = jnp.concatenate(gs, axis=1)
            copies[("u", 0)].wait()
        else:
            g = jnp.dot(xn[...], wg_v[:, pl.ds(f * FC, FC)], preferred_element_type=f32)
        u = jnp.dot(xn[...], wu_v[:, pl.ds(f * FC, FC)], preferred_element_type=f32)
        h = (g * _sigmoid(g) * u).astype(bf16)
        if first:
            copies[("d", 0)].wait()
        dn = jnp.dot(h, wd_v[pl.ds(f * FC, FC), :], preferred_element_type=f32)
        if f == 0:
            acc_v[...] = dn
        elif f == NF - 1:
            accF_v[...] = acc_v[...] + dn
        else:
            acc_v[...] += dn

    def qkv(xn, which=(0, 1, 2)):
        for j in which:
            ref = (q_v, k_v, v_v)[j]
            off = 0 if j == 0 else 16
            for c2 in range(4):
                t = jnp.dot(xn[...], wqkvp_v[:, pl.ds(j * D + c2 * 256, 256)], preferred_element_type=f32)
                if j == 0:
                    t = t * scale
                ref[2 * c2, pl.ds(off, BM), :] = t[:, :128]
                ref[2 * c2 + 1, pl.ds(off, BM), :] = t[:, 128:]

    def att_piece(r0, row0):
        R = 8
        b0 = (lane & 1) != 0
        b1 = (lane & 2) != 0
        def swp(a, bit):
            if USE_PERM:
                return jnp.take_along_axis(a, lane ^ bit, axis=1)
            return jnp.where(b0 if bit == 1 else b1, pltpu.roll(a, bit, 1), pltpu.roll(a, 128 - bit, 1))
        qs = [q_v[c, pl.ds(r0, R), :] for c in range(8)]
        lg = []
        for w0 in range(0, 8, WST):
            grp = []
            for w in range(w0, w0 + WST):
                a = None
                for c in range(8):
                    t = qs[c] * k_v[c, pl.ds(r0 + 16 - 2 * w, R), :]
                    a = t if a is None else a + t
                grp.append(a)
            r1 = [swp(a, 1) for a in grp]
            grp = [a + b for a, b in zip(grp, r1)]
            r2 = [swp(a, 2) for a in grp]
            grp = [a + b for a, b in zip(grp, r2)]
            lg += grp
        if row0 + r0 < 16:
            rows = (row0 + r0) + sub
            lg = [a if w == 0 else jnp.where(rows >= 2 * w, a, -1e9) for w, a in enumerate(lg)]
        m = lg[0]
        for w in range(1, 8):
            m = jnp.maximum(m, lg[w])
        p = [jnp.exp(l - m) for l in lg]
        ssum = p[0]
        for w in range(1, 8):
            ssum = ssum + p[w]
        inv = 1.0 / ssum
        p = [pw * inv for pw in p]
        for c in range(8):
            o = None
            for w in range(8):
                t = p[w] * v_v[c, pl.ds(r0 + 16 - 2 * w, R), :]
                o = t if o is None else o + t
            o_v[pl.ds(r0, R), pl.ds(c * 128, 128)] = o.astype(bf16)

    def wo_epi(row0, last):
        for j in range(D // TC):
            cs = pl.ds(j * TC, TC)
            s = jnp.dot(o_v[...], wop_v[:, cs], preferred_element_type=f32)
            a = accF_v[:, cs]
            res = x_v[pl.ds(row0, BM), cs].astype(f32) + s * (a * _sigmoid(a))
            out_v[:, cs] = res.astype(bf16)
            if last:
                out_copy_cols(row0, j).start()
        if not last:
            out_copy(row0).start()

    k_v[:, 0:16, :] = jnp.zeros((8, 16, 128), f32)
    v_v[:, 0:16, :] = jnp.zeros((8, 16, 128), f32)

    nsep = [0]
    seps = [pltpu.make_async_copy(x_hbm.at[pl.ds(0, 16), pl.ds(0, 128)], sep_v.at[n], sem_s.at[n]) for n in range(NSEP)]
    for c in seps:
        c.start()
    def sep():
        seps[nsep[0]].wait()
        nsep[0] += 1

    xn = (xnA, xnB)
    if True:
        pr = BM // X0P
        for p in range(X0P):
            copies[("x0", p)].wait()
            ln_rows(p * pr, xn[0], p * pr, pr)

    for f in range(FA):
        if True:
            if f == 0:
                ffn_chunk(0, xn[0], first=True)
            else:
                if f >= 2:
                    copies[("qkv", f - 2)].wait()
                for kind in ("g", "u", "d"):
                    copies[(kind, f)].wait()
                ffn_chunk(f, xn[0])
                if f >= 2:
                    perm_qkv(f - 2)
    if True:
        copies[("qkv", 2)].wait()
        qkv(xn[0], (0, 1))
        perm_qkv(2)
    if True:
        copies[("wo", 0)].wait()
        qkv(xn[0], (2,))

    for i in range(NB_GEN):
        row0 = i * BM
        last = i + 1 == NB
        if True:
            if i == 0:
                for f in range(FA, NF):
                    for kind in ("g", "u", "d"):
                        copies[(kind, f)].wait()
            if not last:
                copies[("x", i + 1)].wait()
            else:
                sep()
            for f in range(FA, NF):
                ffn_chunk(f, xn[i % 2])
            for t in range(BM // 8):
                att_piece(t * 8, row0)
            if not last:
                layernorm(row0 + BM, xn[(i + 1) % 2])
                ffn_chunk(0, xn[(i + 1) % 2])
        if True:
            if i == 0:
                sep()
            else:
                out_copy(row0 - BM).wait()
            if not last:
                k_v[:, pl.ds(0, 16), :] = k_v[:, pl.ds(BM, 16), :]
                v_v[:, pl.ds(0, 16), :] = v_v[:, pl.ds(BM, 16), :]
                ffn_chunk(1, xn[(i + 1) % 2])
            if i == 0:
                perm_wo()
            wo_epi(row0, last)
            if not last:
                for f in range(2, FA):
                    ffn_chunk(f, xn[(i + 1) % 2])
                qkv(xn[(i + 1) % 2])
    for j in range(D // TC):
        out_copy_cols(S - BM, j).wait()


@jax.jit
def pallas_recurrent_scan__sliding_local_dilated__swiglu_ffn__prompt_kernel(
    A_x, A_wqkv, A_wo, B_x, B_w_gate, B_w_up, B_w_down):
    B, S, D = A_x.shape
    F = B_w_gate.shape[1]
    x2 = A_x.reshape(S, D)
    bf = jnp.bfloat16
    f32 = jnp.float32
    NB = S // BM
    NF = F // FC
    out = pl.pallas_call(
        kernel,
        out_shape=jax.ShapeDtypeStruct((S, D), bf),
        in_specs=[pl.BlockSpec(memory_space=pl.ANY)] * 6,
        out_specs=pl.BlockSpec(memory_space=pl.ANY),
        scratch_shapes=[
            pltpu.VMEM((S, D), bf), pltpu.VMEM((BM, D), bf), pltpu.VMEM((BM, D), bf),
            pltpu.VMEM((D, 3 * D), bf), pltpu.VMEM((D, 3 * D), bf),
            pltpu.VMEM((D, D), bf), pltpu.VMEM((D, D), bf),
            pltpu.VMEM((D, F), bf), pltpu.VMEM((D, F), bf), pltpu.VMEM((F, D), bf),
            pltpu.VMEM((8, BM, 128), f32),
            pltpu.VMEM((8, BM + 16, 128), f32),
            pltpu.VMEM((8, BM + 16, 128), f32),
            pltpu.VMEM((BM, D), bf), pltpu.VMEM((BM, D), f32), pltpu.VMEM((BM, D), f32),
            pltpu.VMEM((BM, D), bf),
            pltpu.VMEM((NSEP, 16, 128), bf),
            pltpu.SemaphoreType.DMA((NB + 4 + 3 * NF + 2 + X0P,)), pltpu.SemaphoreType.DMA((1 + D // TC,)), pltpu.SemaphoreType.DMA((NSEP,)),
        ],
        compiler_params=pltpu.CompilerParams(vmem_limit_bytes=110 * 1024 * 1024),
    )(x2, A_wqkv, A_wo, B_w_gate, B_w_up, B_w_down)
    return out.reshape(B, S, D)
```

```python
import jax
import jax.numpy as jnp
from jax import lax
import jax.experimental.pallas as pl
import jax.experimental.pallas.tpu as pltpu

BM = 512
FC = 512
FA = 4
NZ = 2
HEADS = 32
WINDOW = 8
DILATION = 2
HALO = 16
X0P = 4
NSEP = 3
G0_PIECES = ((0, 128), (128, 128), (256, 256))
WGROUPS = (2, 1, 1, 2, 1, 1)
WGROUPS_LAST = (2, 2, 2, 2)
PERM_ROWS = 32
STRIP = 16

_F32 = jnp.float32
_BF16 = jnp.bfloat16
_CIDX = (0, None, 1, 2, None, 3, 4)


def _unrolled(n, body):
    def step(i, carry):
        body(i)
        return carry
    lax.fori_loop(0, n, step, 0, unroll=n)


def _sigmoid(x):
    return 0.5 * jnp.tanh(0.5 * x) + 0.5


def _swap(a, b, bit, idx, axis, size):
    hi = (idx & bit) != 0
    return jnp.where(hi, pltpu.roll(b, bit, axis), a), jnp.where(hi, b, pltpu.roll(a, size - bit, axis))


def _a_combos(a11, a12, a21, a22):
    return (a11 + a22, a21 + a22, a11, a22, a11 + a12, a21 - a11, a12 - a22)


def _b_combos(b11, b12, b21, b22):
    return (b11 + b22, b12 - b22, b21 - b11, b11 + b12, b21 + b22)


def _strassen(a, b, order=(1, 4, 0, 2, 3, 5, 6)):
    m = {i: jnp.dot(a(i), b(i), preferred_element_type=_F32) for i in order}
    return (m[0] + m[3] - m[4] + m[6], m[2] + m[4], m[1] + m[3], m[0] - m[1] + m[2] + m[5])


def _kernel(x_hbm, wqkv_hbm, wo_hbm, wg_hbm, wu_hbm, wd_hbm, out_hbm,
            x_v, xn0_v, xa_even, xa_odd, wqkv_v, wqkvp_v, wo_v, wop_v, wg_v, wu_v, wd_v,
            cg_v, cu_v, cd_v, cq_v, cw_v, st_v,
            q_v, k_v, v_v, o_v, acc_v, ffn_v, out_v,
            sep_v, sem_in, sem_out, sem_sep):
    S, D = x_v.shape
    F = wg_v.shape[1]
    NB, NF = S // BM, F // FC
    H, DH, FH = BM // 2, D // 2, FC // 2
    NC = D // 128
    scale = float(D // HEADS) ** -0.5
    xa = (xa_even, xa_odd)

    def chunk_keys(f):
        return [("g", f), ("u", f), ("d", f)]

    order = [("x0", p) for p in range(X0P)] + [("g0", j) for j in range(len(G0_PIECES))] + [("u", 0), ("d", 0)]
    for f in range(1, FA):
        order += [("qkv", f - 2)] * (f >= 2) + chunk_keys(f)
    order += [("qkv", 2), ("wo", 0), ("x", 1)]
    for f in range(FA, NF):
        order += chunk_keys(f)
    order += [("x", j) for j in range(2, NB)]
    copies = {}
    for n, (kind, j) in enumerate(order):
        if kind == "x0":
            src, dst = (r.at[pl.ds(j * (BM // X0P), BM // X0P), :] for r in (x_hbm, x_v))
        elif kind == "x":
            src, dst = (r.at[pl.ds(j * BM, BM), :] for r in (x_hbm, x_v))
        elif kind == "g0":
            src, dst = (r.at[:, pl.ds(*G0_PIECES[j])] for r in (wg_hbm, wg_v))
        elif kind == "g":
            src, dst = (r.at[:, pl.ds(j * FC, FC)] for r in (wg_hbm, wg_v))
        elif kind == "u":
            src, dst = (r.at[:, pl.ds(j * FC, FC)] for r in (wu_hbm, wu_v))
        elif kind == "d":
            src, dst = (r.at[pl.ds(j * FC, FC), :] for r in (wd_hbm, wd_v))
        elif kind == "qkv":
            src, dst = (r.at[:, pl.ds(j * D, D)] for r in (wqkv_hbm, wqkv_v))
        else:
            src, dst = wo_hbm, wo_v
        copies[(kind, j)] = pltpu.make_async_copy(src, dst, sem_in.at[n])
    for key in order:
        copies[key].start()

    def out_copy(row0):
        return pltpu.make_async_copy(out_v, out_hbm.at[pl.ds(row0, BM), :], sem_out.at[0])

    def out_copy_quad(row0, n):
        cs = pl.ds((n % 2) * DH, DH)
        return pltpu.make_async_copy(out_v.at[pl.ds((n // 2) * H, H), cs],
                                     out_hbm.at[pl.ds(row0 + (n // 2) * H, H), cs], sem_out.at[1 + n])

    lane = lax.broadcasted_iota(jnp.int32, (8, 128), 1)
    sub = lax.broadcasted_iota(jnp.int32, (8, 128), 0)

    def permute_qkv(j):
        lane_p = lax.broadcasted_iota(jnp.int32, (PERM_ROWS // 2, 128), 1)

        def step(g):
            rows = pl.ds(pl.multiple_of(g * PERM_ROWS, PERM_ROWS), PERM_ROWS)
            cols = [pltpu.bitcast(wqkv_v[rows, pl.ds(j * D + c * 128, 128)], jnp.uint32) for c in range(NC)]
            for col_bit, lane_bit in ((4, 16), (2, 8), (1, 4)):
                for c in range(NC):
                    if c & col_bit == 0:
                        cols[c], cols[c | col_bit] = _swap(cols[c], cols[c | col_bit], lane_bit, lane_p, 1, 128)
            for c in range(NC):
                wqkvp_v[rows, pl.ds(j * D + c * 128, 128)] = pltpu.bitcast(cols[c], _BF16)
        _unrolled(D // PERM_ROWS, step)

    def permute_wo():
        def step(g):
            h4, h10, d4 = g >> 3, (g >> 1) & 3, g & 1
            for c in range(NC):
                cs = pl.ds(c * 128, 128)
                t = [pltpu.bitcast(wo_v[pl.ds(pl.multiple_of((h4 * 32 + n * 8 + h10 * 2 + d4) * 16, 16), 16), cs],
                                   jnp.uint32) for n in range(4)]
                t[0], t[2] = _swap(t[0], t[2], 4, sub, 0, 8)
                t[1], t[3] = _swap(t[1], t[3], 4, sub, 0, 8)
                t[0], t[1] = _swap(t[0], t[1], 2, sub, 0, 8)
                t[2], t[3] = _swap(t[2], t[3], 2, sub, 0, 8)
                for n in range(4):
                    wop_v[pl.ds(pl.multiple_of((d4 * 32 + n * 8 + h10 * 2 + h4) * 16, 16), 16), cs] = (
                        pltpu.bitcast(t[n], _BF16))
        _unrolled(16, step)

    def row_stats(rows):
        xb = x_v[rows, :].astype(_F32)
        mu = jnp.mean(xb, axis=-1, keepdims=True)
        xc = xb - mu
        var = jnp.mean(xc * xc, axis=-1, keepdims=True)
        return xc, mu, lax.rsqrt(var + 1e-5)

    def store_stats(rows, mu, rstd):
        st_v[0, rows, :] = jnp.broadcast_to(mu, (mu.shape[0], 128))
        st_v[1, rows, :] = jnp.broadcast_to(rstd, (rstd.shape[0], 128))

    def layernorm_first(r0, n):
        rows = pl.ds(r0, n)
        xc, mu, rstd = row_stats(rows)
        store_stats(rows, mu, rstd)
        xn0_v[rows, :] = (xc * rstd).astype(_BF16)

    def layernorm_stats(row0):
        def step(g):
            r = pl.multiple_of(g * STRIP, STRIP)
            _, mu, rstd = row_stats(pl.ds(row0 + r, STRIP))
            store_stats(pl.ds(r, STRIP), mu, rstd)
        _unrolled(BM // STRIP, step)

    def layernorm_operands(row0, dst):
        def normalised(r):
            mu, rstd = st_v[0, pl.ds(r, STRIP), :], st_v[1, pl.ds(r, STRIP), :]
            return jnp.concatenate(
                [(x_v[pl.ds(row0 + r, STRIP), pl.ds(c * 128, 128)].astype(_F32) - mu) * rstd for c in range(NC)], axis=1)

        def step(g):
            r = pl.multiple_of(g * STRIP, STRIP)
            top, bot = normalised(r), normalised(H + r)
            for i, c in enumerate(_a_combos(top[:, :DH], top[:, DH:], bot[:, :DH], bot[:, DH:])):
                dst[i, pl.ds(r, STRIP), :] = c.astype(_BF16)
        _unrolled(H // STRIP, step)

    def quadrants(ref, r0, rn, c0, cn):
        return [ref.at[pl.ds(r0 + (n // 2) * rn, rn), pl.ds(c0 + (n % 2) * cn, cn)] for n in range(4)]

    def prepare(quads, dst):
        def step(g):
            rows = pl.ds(pl.multiple_of(g * STRIP, STRIP), STRIP)
            for i, c in enumerate(_b_combos(*[q[rows, :].astype(_F32) for q in quads])):
                dst[i, rows, :] = c.astype(_BF16)
        _unrolled(quads[0].shape[0] // STRIP, step)

    def right(quads, sums):
        return lambda i: quads[0][...] if i == 1 else quads[3][...] if i == 4 else sums[_CIDX[i]]

    def gate_q(f): return quadrants(wg_v, 0, DH, f * FC, FH)
    def up_q(f): return quadrants(wu_v, 0, DH, f * FC, FH)
    def down_q(f): return quadrants(wd_v, f * FC, FH, 0, DH)
    def qkv_q(j): return quadrants(wqkvp_v, 0, DH, j * D, DH)

    def prepare_ffn(f):
        prepare(gate_q(f), cg_v.at[f])
        prepare(up_q(f), cu_v.at[f])
        prepare(down_q(f), cd_v.at[f])

    def ffn_first_chunk():
        gs = []
        for j, piece in enumerate(G0_PIECES):
            copies[("g0", j)].wait()
            gs.append(jnp.dot(xn0_v[...], wg_v[:, pl.ds(*piece)], preferred_element_type=_F32))
        g = jnp.concatenate(gs, axis=1)
        copies[("u", 0)].wait()
        u = jnp.dot(xn0_v[...], wu_v[:, pl.ds(0, FC)], preferred_element_type=_F32)
        h = (g * _sigmoid(g) * u).astype(_BF16)
        copies[("d", 0)].wait()
        acc_v[...] = jnp.dot(h, wd_v[pl.ds(0, FC), :], preferred_element_type=_F32)

    def ffn_chunk(f, left):
        g = _strassen(lambda i: left[i], right(gate_q(f), cg_v.at[f]))
        u = _strassen(lambda i: left[i], right(up_q(f), cu_v.at[f]))
        h = _a_combos(*[gg * _sigmoid(gg) * uu for gg, uu in zip(g, u)])
        h = [c.astype(_BF16) for c in h]
        for n, c in enumerate(_strassen(lambda i: h[i], right(down_q(f), cd_v.at[f]))):
            idx = (pl.ds((n // 2) * H, H), pl.ds((n % 2) * DH, DH))
            if f == 0:
                acc_v[idx] = c
            elif f == NF - 1:
                ffn_v[idx] = acc_v[idx] + c
            else:
                acc_v[idx] += c

    def project_qkv(left, which=(0, 1, 2), first=False):
        for j in which:
            if first:
                prepare(qkv_q(j), cq_v.at[j])
            ref, off = ((q_v, 0), (k_v, HALO), (v_v, HALO))[j]
            for n, t in enumerate(_strassen(lambda i: left[i], right(qkv_q(j), cq_v.at[j]))):
                if j == 0:
                    t = t * scale
                for c in range(NC // 2):
                    ref[(n % 2) * (NC // 2) + c, pl.ds(off + (n // 2) * H, H), :] = t[:, c * 128:(c + 1) * 128]

    def attend_rows(r0, groups, first_rows=None):
        def lane_pair(a, bit):
            return jnp.where((lane & bit) != 0, pltpu.roll(a, bit, 1), pltpu.roll(a, 128 - bit, 1))

        def window(ref, c, w):
            return ref[c, pl.ds(r0 + HALO - DILATION * w, 8), :]

        q = [q_v[c, pl.ds(r0, 8), :] for c in range(NC)]
        logits, w0 = [], 0
        for size in groups:
            part = []
            for w in range(w0, w0 + size):
                a = q[0] * window(k_v, 0, w)
                for c in range(1, NC):
                    a = a + q[c] * window(k_v, c, w)
                part.append(a)
            for bit in (1, 2):
                other = [lane_pair(a, bit) for a in part]
                part = [a + b for a, b in zip(part, other)]
            logits += part
            w0 += size
        if first_rows is not None:
            logits = [a if w == 0 else jnp.where(first_rows + sub >= DILATION * w, a, -1e9)
                      for w, a in enumerate(logits)]
        m = logits[0]
        for a in logits[1:]:
            m = jnp.maximum(m, a)
        p = [jnp.exp(a - m) for a in logits]
        total = p[0]
        for a in p[1:]:
            total = total + a
        inv = 1.0 / total
        p = [a * inv for a in p]
        for c in range(NC):
            o = p[0] * window(v_v, c, 0)
            for w in range(1, WINDOW):
                o = o + p[w] * window(v_v, c, w)
            o_v[pl.ds(r0, 8), pl.ds(c * 128, 128)] = o.astype(_BF16)

    def attend(i):
        groups = WGROUPS_LAST if i == NB - 1 else WGROUPS
        t0 = 0
        if i == 0:
            t0 = HALO // 8
            for t in range(t0):
                attend_rows(8 * t, groups, first_rows=8 * t)
        _unrolled(BM // 8 - t0, lambda t: attend_rows(pl.multiple_of((t0 + t) * 8, 8), groups))

    def project_out(i):
        row0, quads = i * BM, quadrants(wop_v, 0, DH, 0, DH)
        if i == 0:
            permute_wo()
            prepare(quads, cw_v)
        o = _a_combos(*[o_v[pl.ds((n // 2) * H, H), pl.ds((n % 2) * DH, DH)].astype(_F32) for n in range(4)])
        o = [c.astype(_BF16) for c in o]
        s = _strassen(lambda n: o[n], right(quads, cw_v), order=(2, 4, 1, 3, 0, 6, 5))
        for n in (1, 2, 0, 3):
            rows, cs = pl.ds((n // 2) * H, H), pl.ds((n % 2) * DH, DH)
            a = ffn_v[rows, cs]
            res = x_v[pl.ds(row0 + (n // 2) * H, H), cs].astype(_F32) + s[n] * (a * _sigmoid(a))
            out_v[rows, cs] = res.astype(_BF16)
            if i == NB - 1:
                out_copy_quad(row0, n).start()
        if i < NB - 1:
            out_copy(row0).start()

    k_v[:, 0:HALO, :] = jnp.zeros((NC, HALO, 128), _F32)
    v_v[:, 0:HALO, :] = jnp.zeros((NC, HALO, 128), _F32)
    seps = [pltpu.make_async_copy(x_hbm.at[pl.ds(0, 16), pl.ds(0, 128)], sep_v.at[n], sem_sep.at[n])
            for n in range(NSEP)]
    for c in seps:
        c.start()

    for p in range(X0P):
        copies[("x0", p)].wait()
        layernorm_first(p * (BM // X0P), BM // X0P)
    ffn_first_chunk()
    for f in range(1, FA):
        if f >= 2:
            copies[("qkv", f - 2)].wait()
        for key in chunk_keys(f):
            copies[key].wait()
        if f == 1:
            layernorm_operands(0, xa[0])
        prepare_ffn(f)
        ffn_chunk(f, xa[0])
        if f >= 2:
            permute_qkv(f - 2)
    copies[("qkv", 2)].wait()
    project_qkv(xa[0], (0, 1), first=True)
    permute_qkv(2)
    copies[("wo", 0)].wait()
    copies[("x", 1)].wait()
    project_qkv(xa[0], (2,), first=True)
    layernorm_stats(BM)

    for i in range(NB):
        cur, nxt, last = xa[i % 2], xa[(i + 1) % 2], i == NB - 1
        if i == 0:
            for f in range(FA, NF):
                for key in chunk_keys(f):
                    copies[key].wait()
        else:
            seps[i - 1].wait()
        for f in range(FA, NF):
            if i == 0:
                prepare_ffn(f)
            ffn_chunk(f, cur)
        attend(i)
        if not last:
            layernorm_operands((i + 1) * BM, nxt)
            for f in range(NZ):
                if i == 0 and f == 0:
                    prepare_ffn(0)
                ffn_chunk(f, nxt)
        if i + 2 < NB:
            copies[("x", i + 2)].wait()
        if i > 0:
            out_copy((i - 1) * BM).wait()
        if not last:
            k_v[:, pl.ds(0, HALO), :] = k_v[:, pl.ds(BM, HALO), :]
            v_v[:, pl.ds(0, HALO), :] = v_v[:, pl.ds(BM, HALO), :]
            ffn_chunk(NZ, nxt)
        project_out(i)
        if not last:
            for f in range(NZ + 1, FA):
                ffn_chunk(f, nxt)
            project_qkv(nxt)
            if i + 2 < NB:
                layernorm_stats((i + 2) * BM)
    for n in range(4):
        out_copy_quad(S - BM, n).wait()


@jax.jit
def pallas_recurrent_scan__sliding_local_dilated__swiglu_ffn__prompt_kernel(
    A_x: jax.Array,
    A_wqkv: jax.Array,
    A_wo: jax.Array,
    B_x: jax.Array,
    B_w_gate: jax.Array,
    B_w_up: jax.Array,
    B_w_down: jax.Array,
):
    del B_x
    B, S, D = A_x.shape
    F = B_w_gate.shape[1]
    assert B == 1 and D == 1024 and S == (NSEP + 1) * BM and F % FC == 0 and F // FC > FA
    NB, NF = S // BM, F // FC
    n_in = X0P + len(G0_PIECES) + 3 * NF - 1 + 3 + 1 + NB - 1

    def vmem(*shape, dtype=_BF16):
        return pltpu.VMEM(shape, dtype)

    out = pl.pallas_call(
        _kernel,
        out_shape=jax.ShapeDtypeStruct((S, D), A_x.dtype),
        in_specs=[pl.BlockSpec(memory_space=pl.ANY)] * 6,
        out_specs=pl.BlockSpec(memory_space=pl.ANY),
        scratch_shapes=[
            vmem(S, D), vmem(BM, D), vmem(7, BM // 2, D // 2), vmem(7, BM // 2, D // 2),
            vmem(D, 3 * D), vmem(D, 3 * D), vmem(D, D), vmem(D, D), vmem(D, F), vmem(D, F), vmem(F, D),
            vmem(NF, 5, D // 2, FC // 2), vmem(NF, 5, D // 2, FC // 2), vmem(NF, 5, FC // 2, D // 2),
            vmem(3, 5, D // 2, D // 2), vmem(5, D // 2, D // 2), vmem(2, BM, 128, dtype=_F32),
            vmem(D // 128, BM, 128, dtype=_F32), vmem(D // 128, BM + HALO, 128, dtype=_F32),
            vmem(D // 128, BM + HALO, 128, dtype=_F32),
            vmem(BM, D), vmem(BM, D, dtype=_F32), vmem(BM, D, dtype=_F32), vmem(BM, D),
            vmem(NSEP, 16, 128),
            pltpu.SemaphoreType.DMA((n_in,)), pltpu.SemaphoreType.DMA((5,)), pltpu.SemaphoreType.DMA((NSEP,)),
        ],
        compiler_params=pltpu.CompilerParams(vmem_limit_bytes=120 * 1024 * 1024),
    )(A_x.reshape(S, D), A_wqkv, A_wo, B_w_gate, B_w_up, B_w_down)
    return out.reshape(B, S, D)
```
